```python
import os as _os
_os.environ.setdefault('JAX_PLATFORMS', 'cpu')
import jax
import jax.numpy as jnp

def _softmax(x, axis=-1):
    return jax.nn.softmax(x, axis=axis)

def _gelu(x):
    return jax.nn.gelu(x, approximate=True)

def _silu(x):
    return jax.nn.silu(x)

def _sigmoid(x):
    return jax.nn.sigmoid(x)

def _layernorm(x, axis=-1, eps=1e-05):
    m = jnp.mean(x, axis=axis, keepdims=True)
    v = jnp.var(x, axis=axis, keepdims=True)
    return (x - m) / jnp.sqrt(v + eps)

def _scatter_add(tgt, idx, src, axis=0):
    return tgt.at[idx].add(src)

def _segment_sum(src, seg, n):
    return jax.ops.segment_sum(src, seg, n)

class _Rng:

    def __init__(self, key):
        self._k = key

    def _next(self):
        self._k, sub = jax.random.split(self._k)
        return sub

    def normal(self, shape):
        return jax.random.normal(self._next(), shape, dtype=jnp.bfloat16)

    def randint(self, lo, hi, shape):
        return jax.random.randint(self._next(), shape, lo, hi, dtype=jnp.int32)

    def uniform(self, shape, lo=0.0, hi=1.0):
        return jax.random.uniform(self._next(), shape, jnp.bfloat16, lo, hi)

    def permutation(self, n):
        return jax.random.permutation(self._next(), n)
kernel_name = 'adaLN_cond__mha_block__dense_activation_squared_relu__prompt'

def setup_inputs():
    _rng = _Rng(jax.random.key(int.from_bytes(__import__("os").urandom(4), "little")))
    _w = lambda a: (lambda t: t.astype(jnp.bfloat16) if jnp.issubdtype(t.dtype, jnp.floating) else t)(jnp.asarray(a))

    def _A_setup():
        B, S, D, H = (1, 2048, 512, 32)
        return {'x': _w((lambda *s: _rng.normal(s) * 0.05)(B, S, D)), 'wqkv': _w((lambda *s: _rng.normal(s) * 0.1)(D, 3 * D)), 'wo': _w((lambda *s: _rng.normal(s) * 0.05)(D, D))}
    _A_in = _A_setup()

    def _B_setup():
        B, S, D, F = (1, 2048, 512, 1792)
        return {'x': _w((lambda *s: _rng.normal(s) * 0.05)(B, S, D)), 'w1': _w((lambda *s: _rng.normal(s) * 0.05)(D, F)), 'b1': _w((lambda *s: _rng.normal(s) * 0.05)(F)), 'w2': _w((lambda *s: _rng.normal(s) * 0.05)(F, D)), 'b2': _w((lambda *s: _rng.normal(s) * 0.05)(D))}
    _B_in = _B_setup()
    return {'A_x': _A_in['x'], 'A_wqkv': _A_in['wqkv'], 'A_wo': _A_in['wo'], 'B_x': _B_in['x'], 'B_w1': _B_in['w1'], 'B_b1': _B_in['b1'], 'B_w2': _B_in['w2'], 'B_b2': _B_in['b2'], 'c': _w((lambda *s: _rng.normal(s) * 0.05)(1, 512) * 8.0), 'w_mod': _w((lambda *s: _rng.normal(s) * 0.05)(512, 6 * 512) * 512 ** (-0.5) * 8.0)}

def reference(A_x, A_wqkv, A_wo, B_x, B_w1, B_b1, B_w2, B_b2, c, w_mod):

    def _A_ref(x, wqkv, wo):
        B, S, D = x.shape
        H = 32
        Dh = D // H
        qkv = (lambda x, *d: x.transpose(*d))((x @ wqkv).reshape(B, S, 3, H, Dh), 2, 0, 3, 1, 4)
        q, k, v = (qkv[0], qkv[1], qkv[2])
        scores = jnp.einsum('bhqd,bhkd->bhqk', q, k) * Dh ** (-0.5)
        p = _softmax(scores, axis=-1)
        o = jnp.einsum('bhqk,bhkd->bhqd', p, v)
        return (lambda x, *d: x.transpose(*d))(o, 0, 2, 1, 3).reshape(B, S, D) @ wo

    def _B_ref(x, w1, b1, w2, b2):
        h = jnp.einsum('bsd,df->bsf', x, w1) + b1
        zero = jnp.zeros_like(h)
        r = jnp.where(h > zero, h, zero)
        h = r * r
        out = jnp.einsum('bsf,fd->bsd', h, w2) + b2
        return out
    x = A_x
    mod = (_silu(c) @ w_mod).reshape(c.shape[0], 6, 1, -1)
    sa, ca, ga, sb, cb, gb = (mod[:, 0].copy(), mod[:, 1].copy(), mod[:, 2].copy(), mod[:, 3].copy(), mod[:, 4].copy(), mod[:, 5].copy())
    h = _layernorm(x, axis=-1) * (1 + ca) + sa
    x = x + ga * _A_ref(h, A_wqkv, A_wo)
    h = _layernorm(x, axis=-1) * (1 + cb) + sb
    x = x + gb * _B_ref(h, B_w1, B_b1, B_w2, B_b2)
    return x
```

```python
import functools
import jax
import jax.numpy as jnp
from jax import lax
import jax.experimental.pallas as pl
import jax.experimental.pallas.tpu as pltpu

S, D, H, DH, F = 2048, 512, 32, 16, 1792
LOG2E = 1.4426950408889634
EPS = 1e-5


def _ln(x):
    m = jnp.mean(x, axis=-1, keepdims=True)
    xc = x - m
    v = jnp.mean(xc * xc, axis=-1, keepdims=True)
    return xc * lax.rsqrt(v + EPS)


def make_kernel(TQ=256, RC=512):
    NQ = S // TQ

    def kernel(x_ref, wqkv_ref, wo_ref, w1_ref, b1_ref, w2_ref, b2_ref, c_ref, wmod_ref,
               o_ref, k_scr, qt_scr, vt_scr, mod_scr, ot_scr):
        i = pl.program_id(0)

        @pl.when(i == 0)
        def _prologue():
            c = c_ref[...].astype(jnp.float32)
            sc = c * jax.nn.sigmoid(c)
            sc8 = jnp.broadcast_to(sc, (8, D)).astype(jnp.bfloat16)
            mod_scr[...] = jnp.dot(sc8, wmod_ref[...], preferred_element_type=jnp.float32)
            sa = mod_scr[0:1, 0:D]
            ca = mod_scr[0:1, D:2 * D]
            wq_t = wqkv_ref[:, 0:D].astype(jnp.float32).T.astype(jnp.bfloat16)
            wv_t = wqkv_ref[:, 2 * D:3 * D].astype(jnp.float32).T.astype(jnp.bfloat16)
            wk = wqkv_ref[:, D:2 * D]
            row = lax.broadcasted_iota(jnp.int32, (DH, RC), 0)
            ones_blk = jnp.where(row == 0, 1.0, 0.0).astype(jnp.bfloat16)
            for r in range(S // RC):
                xr = x_ref[0, r * RC:(r + 1) * RC, :].astype(jnp.float32)
                h = (_ln(xr) * (1.0 + ca) + sa).astype(jnp.bfloat16)
                kk = jnp.dot(h, wk, preferred_element_type=jnp.float32).astype(jnp.bfloat16)
                for g in range(4):
                    k_scr[g, r * RC:(r + 1) * RC, :] = kk[:, g * 128:(g + 1) * 128]
                qt = lax.dot_general(wq_t, h, (((1,), (1,)), ((), ())),
                                     preferred_element_type=jnp.float32)
                qt = (qt * (DH ** -0.5 * LOG2E)).astype(jnp.bfloat16)
                for b in range(RC // TQ):
                    qt_scr[r * (RC // TQ) + b] = qt[:, b * TQ:(b + 1) * TQ]
                vt = lax.dot_general(wv_t, h, (((1,), (1,)), ((), ())),
                                     preferred_element_type=jnp.float32).astype(jnp.bfloat16)
                for hh in range(H):
                    vt_scr[hh, 0:DH, r * RC:(r + 1) * RC] = vt[hh * DH:(hh + 1) * DH, :]
                    vt_scr[hh, DH:2 * DH, r * RC:(r + 1) * RC] = ones_blk

        rowh = lax.broadcasted_iota(jnp.int32, (128, TQ), 0) // DH

        def head_body(hh, carry):
            g = hh // 8
            j = hh % 8
            qg = qt_scr[i, pl.ds(pl.multiple_of(g * 128, 128), 128), :]
            w = jnp.where(rowh == j, qg, jnp.zeros_like(qg))
            s = jnp.dot(k_scr[g], w, preferred_element_type=jnp.float32)
            m = jnp.max(s, axis=0, keepdims=True)
            p = jnp.exp2(s - m).astype(jnp.bfloat16)
            o = jnp.dot(vt_scr[hh], p, preferred_element_type=jnp.float32)
            on = o[0:DH, :] / o[DH:DH + 1, :]
            ot_scr[pl.ds(pl.multiple_of(hh * DH, DH), DH), :] = on
            return carry

        lax.fori_loop(0, H, head_body, 0)

        ga = mod_scr[0:1, 2 * D:3 * D]
        sb = mod_scr[0:1, 3 * D:4 * D]
        cb = mod_scr[0:1, 4 * D:5 * D]
        gb = mod_scr[0:1, 5 * D:6 * D]
        o_att = ot_scr[...].T.astype(jnp.bfloat16)
        a = jnp.dot(o_att, wo_ref[...], preferred_element_type=jnp.float32)
        q0 = pl.multiple_of(i * TQ, TQ)
        x = x_ref[0, pl.ds(q0, TQ), :].astype(jnp.float32)
        x1 = x + ga * a
        h2 = (_ln(x1) * (1.0 + cb) + sb).astype(jnp.bfloat16)
        u = jnp.dot(h2, w1_ref[...], preferred_element_type=jnp.float32) + b1_ref[...].astype(jnp.float32)
        u = jnp.maximum(u, 0.0)
        u = (u * u).astype(jnp.bfloat16)
        y = jnp.dot(u, w2_ref[...], preferred_element_type=jnp.float32) + b2_ref[...].astype(jnp.float32)
        o_ref[0] = (x1 + gb * y).astype(o_ref.dtype)

    def full(shape):
        n = len(shape)
        return pl.BlockSpec(shape, lambda i: (0,) * n)

    @jax.jit
    def f(A_x, A_wqkv, A_wo, B_x, B_w1, B_b1, B_w2, B_b2, c, w_mod):
        b1 = B_b1.reshape(1, F)
        b2 = B_b2.reshape(1, D)
        return pl.pallas_call(
            kernel,
            grid=(NQ,),
            in_specs=[full((1, S, D)), full((D, 3 * D)), full((D, D)), full((D, F)), full((1, F)),
                      full((F, D)), full((1, D)), full((1, D)), full((D, 6 * D))],
            out_specs=pl.BlockSpec((1, TQ, D), lambda i: (0, i, 0)),
            out_shape=jax.ShapeDtypeStruct((1, S, D), jnp.bfloat16),
            scratch_shapes=[
                pltpu.VMEM((4, S, 128), jnp.bfloat16),
                pltpu.VMEM((NQ, D, TQ), jnp.bfloat16),
                pltpu.VMEM((H, 2 * DH, S), jnp.bfloat16),
                pltpu.VMEM((8, 6 * D), jnp.float32),
                pltpu.VMEM((D, TQ), jnp.float32),
            ],
            compiler_params=pltpu.CompilerParams(
                dimension_semantics=("arbitrary",), vmem_limit_bytes=100 * 1024 * 1024),
        )(A_x, A_wqkv, A_wo, B_w1, b1, B_w2, b2, c, w_mod)

    return f


_impl = make_kernel()


@jax.jit
def pallas_adaLN_cond__mha_block__dense_activation_squared_relu__prompt_kernel(A_x, A_wqkv, A_wo, B_x, B_w1, B_b1, B_w2, B_b2, c, w_mod):
    return _impl(A_x, A_wqkv, A_wo, B_x, B_w1, B_b1, B_w2, B_b2, c, w_mod)
```

```python
import functools
import jax
import jax.numpy as jnp
from jax import lax
import jax.experimental.pallas as pl
import jax.experimental.pallas.tpu as pltpu

S, D, H, DH, F = 2048, 512, 32, 16, 1792
LOG2E = 1.4426950408889634
EPS = 1e-5


def _ln(x):
    m = jnp.mean(x, axis=-1, keepdims=True)
    xc = x - m
    v = jnp.mean(xc * xc, axis=-1, keepdims=True)
    return xc * lax.rsqrt(v + EPS)


def make_kernel(TQ=512, RC=512, TK=128, NIT=None, ONED=True):
    NQ = S // TQ
    NC = S // TK
    NR = S // RC
    if NIT is None:
        NIT = H // 2 - 1

    def kernel(x_hbm, wqkv_hbm, wo_hbm, w1_hbm, b1_ref, w2_hbm, b2_ref, c_ref, wmod_hbm,
               o_ref, x_ref, wqkv_ref, wo_ref, w1_ref, w2_ref, wmod_ref, sems,
               k_scr, qt_scr, vt_scr, mod_scr, ot_scr, sa_scr, sb_scr, ma_scr, mb_scr):
        i = pl.program_id(0)

        def x_copy(r):
            return pltpu.make_async_copy(x_hbm.at[0, r * RC:(r + 1) * RC, :],
                                         x_ref.at[r * RC:(r + 1) * RC, :], sems.at[r])

        cp_mod_a = pltpu.make_async_copy(wmod_hbm.at[:, 0:2 * D], wmod_ref.at[:, 0:2 * D], sems.at[NR])
        cp_mod_b = pltpu.make_async_copy(wmod_hbm.at[:, 2 * D:6 * D], wmod_ref.at[:, 2 * D:6 * D],
                                         sems.at[NR + 1])
        cp_qkv = pltpu.make_async_copy(wqkv_hbm, wqkv_ref, sems.at[NR + 2])
        cp_wo = pltpu.make_async_copy(wo_hbm, wo_ref, sems.at[NR + 3])
        cp_w1 = pltpu.make_async_copy(w1_hbm, w1_ref, sems.at[NR + 4])
        cp_w2 = pltpu.make_async_copy(w2_hbm, w2_ref, sems.at[NR + 5])

        rowh = lax.broadcasted_iota(jnp.int32, (128, TQ), 0) // DH

        def step(qb, ha, hb, s_a, m_a, s_b, m_b):
            if ha is not None:
                g = ha // 8
                j = ha % 8
                if isinstance(g, int):
                    qg = qt_scr[qb, g * 128:(g + 1) * 128, :]
                else:
                    qg = qt_scr[qb, pl.ds(pl.multiple_of(g * 128, 128), 128), :]
                w = jnp.where(rowh == j, qg, jnp.zeros_like(qg))
            if hb is not None:
                mb = m_b[...]
            mx = None
            o = None
            l = None
            for c in range(NC):
                if ha is not None:
                    s = jnp.dot(k_scr[g, c * TK:(c + 1) * TK, :], w,
                                preferred_element_type=jnp.float32)
                    s_a[c * TK:(c + 1) * TK, :] = s
                    mc = jnp.max(s.reshape(TK // 8, 8, TQ), axis=0)
                    mx = mc if mx is None else jnp.maximum(mx, mc)
                if hb is not None:
                    p = jnp.exp2(s_b[c * TK:(c + 1) * TK, :] - mb)
                    lc = jnp.sum(p.reshape(TK // 8, 8, TQ), axis=0)
                    l = lc if l is None else l + lc
                    oc = jnp.dot(vt_scr[hb, :, c * TK:(c + 1) * TK], p.astype(jnp.bfloat16),
                                 preferred_element_type=jnp.float32)
                    o = oc if o is None else o + oc
            if ha is not None:
                m_a[...] = jnp.max(mx, axis=0, keepdims=True)
            if hb is not None:
                on = o / jnp.sum(l, axis=0, keepdims=True)
                if isinstance(hb, int):
                    ot_scr[hb * DH:(hb + 1) * DH, :] = on
                else:
                    ot_scr[pl.ds(pl.multiple_of(hb * DH, DH), DH), :] = on

        @pl.when(i == 0)
        def _prologue():
            cp_mod_a.start()
            x_copy(0).start()
            cp_qkv.start()
            for r in range(1, NR):
                x_copy(r).start()
            cp_mod_b.start()
            cp_wo.start()
            cp_w1.start()
            cp_w2.start()

            c = c_ref[...].astype(jnp.float32)
            sc = c * jax.nn.sigmoid(c)
            sc8 = jnp.broadcast_to(sc, (8, D)).astype(jnp.bfloat16)
            cp_mod_a.wait()
            mod_scr[:, 0:2 * D] = jnp.dot(sc8, wmod_ref[:, 0:2 * D], preferred_element_type=jnp.float32)
            sa = mod_scr[0:1, 0:D]
            ca = mod_scr[0:1, D:2 * D]
            cp_qkv.wait()
            wq_t = wqkv_ref[:, 0:D].astype(jnp.float32).T.astype(jnp.bfloat16)
            wv_t = wqkv_ref[:, 2 * D:3 * D].astype(jnp.float32).T.astype(jnp.bfloat16)
            wk = wqkv_ref[:, D:2 * D]
            for r in range(NR):
                x_copy(r).wait()
                xr = x_ref[r * RC:(r + 1) * RC, :].astype(jnp.float32)
                h = (_ln(xr) * (1.0 + ca) + sa).astype(jnp.bfloat16)
                kk = jnp.dot(h, wk, preferred_element_type=jnp.float32).astype(jnp.bfloat16)
                for g in range(4):
                    k_scr[g, r * RC:(r + 1) * RC, :] = kk[:, g * 128:(g + 1) * 128]
                qt = lax.dot_general(wq_t, h, (((1,), (1,)), ((), ())),
                                     preferred_element_type=jnp.float32)
                qt = (qt * (DH ** -0.5 * LOG2E)).astype(jnp.bfloat16)
                if RC >= TQ:
                    for b in range(RC // TQ):
                        qt_scr[r * (RC // TQ) + b] = qt[:, b * TQ:(b + 1) * TQ]
                else:
                    qt_scr[(r * RC) // TQ, :, (r * RC) % TQ:(r * RC) % TQ + RC] = qt
                vt = lax.dot_general(wv_t, h, (((1,), (1,)), ((), ())),
                                     preferred_element_type=jnp.float32).astype(jnp.bfloat16)
                for hh in range(H):
                    vt_scr[hh, :, r * RC:(r + 1) * RC] = vt[hh * DH:(hh + 1) * DH, :]
            cp_mod_b.wait()
            mod_scr[:, 2 * D:6 * D] = jnp.dot(sc8, wmod_ref[:, 2 * D:6 * D],
                                              preferred_element_type=jnp.float32)
            step(0, 0, None, sa_scr, ma_scr, None, None)

        def pair_body(t, carry):
            h0 = 2 * t
            step(i, h0 + 1, h0, sb_scr, mb_scr, sa_scr, ma_scr)
            step(i, h0 + 2, h0 + 1, sa_scr, ma_scr, sb_scr, mb_scr)
            return carry

        lax.fori_loop(0, NIT, pair_body, 0)
        step(i, H - 1, H - 2, sb_scr, mb_scr, sa_scr, ma_scr)

        @pl.when(i < NQ - 1)
        def _():
            step(i + 1, 0, H - 1, sa_scr, ma_scr, sb_scr, mb_scr)

        @pl.when(i == NQ - 1)
        def _():
            step(None, None, H - 1, None, None, sb_scr, mb_scr)

        @pl.when(i == 0)
        def _():
            cp_wo.wait()
            cp_w1.wait()
            cp_w2.wait()

        ga = mod_scr[0:1, 2 * D:3 * D]
        sb = mod_scr[0:1, 3 * D:4 * D]
        cb = mod_scr[0:1, 4 * D:5 * D]
        gb = mod_scr[0:1, 5 * D:6 * D]
        o_att = ot_scr[...].T.astype(jnp.bfloat16)
        a = jnp.dot(o_att, wo_ref[...], preferred_element_type=jnp.float32)
        q0 = pl.multiple_of(i * TQ, TQ)
        x = x_ref[pl.ds(q0, TQ), :].astype(jnp.float32)
        x1 = x + ga * a
        h2 = (_ln(x1) * (1.0 + cb) + sb).astype(jnp.bfloat16)
        b1 = b1_ref[...].astype(jnp.float32).reshape(1, F)
        b2 = b2_ref[...].astype(jnp.float32).reshape(1, D)
        u = jnp.dot(h2, w1_ref[...], preferred_element_type=jnp.float32) + b1
        u = jnp.maximum(u, 0.0)
        u = (u * u).astype(jnp.bfloat16)
        y = jnp.dot(u, w2_ref[...], preferred_element_type=jnp.float32) + b2
        o_ref[0] = (x1 + gb * y).astype(o_ref.dtype)

    def full(shape):
        n = len(shape)
        return pl.BlockSpec(shape, lambda i: (0,) * n)

    hbm = pl.BlockSpec(memory_space=pl.ANY)

    @jax.jit
    def f(A_x, A_wqkv, A_wo, B_x, B_w1, B_b1, B_w2, B_b2, c, w_mod):
        if ONED:
            b1, b2 = B_b1, B_b2
        else:
            b1 = B_b1.reshape(1, F)
            b2 = B_b2.reshape(1, D)
        return pl.pallas_call(
            kernel,
            grid=(NQ,),
            in_specs=[hbm, hbm, hbm, hbm, full(b1.shape), hbm, full(b2.shape), full((1, D)), hbm],
            out_specs=pl.BlockSpec((1, TQ, D), lambda i: (0, i, 0)),
            out_shape=jax.ShapeDtypeStruct((1, S, D), jnp.bfloat16),
            scratch_shapes=[
                pltpu.VMEM((S, D), jnp.bfloat16),
                pltpu.VMEM((D, 3 * D), jnp.bfloat16),
                pltpu.VMEM((D, D), jnp.bfloat16),
                pltpu.VMEM((D, F), jnp.bfloat16),
                pltpu.VMEM((F, D), jnp.bfloat16),
                pltpu.VMEM((D, 6 * D), jnp.bfloat16),
                pltpu.SemaphoreType.DMA((NR + 6,)),
                pltpu.VMEM((4, S, 128), jnp.bfloat16),
                pltpu.VMEM((NQ, D, TQ), jnp.bfloat16),
                pltpu.VMEM((H, DH, S), jnp.bfloat16),
                pltpu.VMEM((8, 6 * D), jnp.float32),
                pltpu.VMEM((D, TQ), jnp.float32),
                pltpu.VMEM((S, TQ), jnp.float32),
                pltpu.VMEM((S, TQ), jnp.float32),
                pltpu.VMEM((1, TQ), jnp.float32),
                pltpu.VMEM((1, TQ), jnp.float32),
            ],
            compiler_params=pltpu.CompilerParams(
                dimension_semantics=("arbitrary",), vmem_limit_bytes=100 * 1024 * 1024),
        )(A_x, A_wqkv, A_wo, B_w1, b1, B_w2, b2, c, w_mod)

    return f


_impl = make_kernel()


@jax.jit
def pallas_adaLN_cond__mha_block__dense_activation_squared_relu__prompt_kernel(A_x, A_wqkv, A_wo, B_x, B_w1, B_b1, B_w2, B_b2, c, w_mod):
    return _impl(A_x, A_wqkv, A_wo, B_x, B_w1, B_b1, B_w2, B_b2, c, w_mod)
```

```python
import functools
import jax
import jax.numpy as jnp
from jax import lax
import jax.experimental.pallas as pl
import jax.experimental.pallas.tpu as pltpu

S, D, H, DH, F = 2048, 512, 32, 16, 1792
LOG2E = 1.4426950408889634
EPS = 1e-5


def _ln(x):
    m = jnp.mean(x, axis=-1, keepdims=True)
    xc = x - m
    v = jnp.mean(xc * xc, axis=-1, keepdims=True)
    return xc * lax.rsqrt(v + EPS)


def make_kernel(TQ=512, RC=512, TK=128, NIT=None, ONED=True, U=2, SKEW=0, G=2):
    NQ = S // TQ
    NC = S // TK
    NR = S // RC
    if NIT is None:
        NIT = H // (2 * G)

    def kernel(x_hbm, wqkv_hbm, wo_hbm, w1_hbm, b1_ref, w2_hbm, b2_ref, c_ref, wmod_hbm,
               o_ref, x_ref, wqkv_ref, wo_ref, w1_ref, w2_ref, wmod_ref, sems,
               k_scr, qt_scr, vt_scr, mod_scr, ot_scr, *sm_scr):
        bufs = [(sm_scr[2 * b], sm_scr[2 * b + 1]) for b in range(2 * G)]
        i = pl.program_id(0)

        def x_copy(r):
            return pltpu.make_async_copy(x_hbm.at[0, r * RC:(r + 1) * RC, :],
                                         x_ref.at[r * RC:(r + 1) * RC, :], sems.at[r])

        cp_mod_a = pltpu.make_async_copy(wmod_hbm.at[:, 0:2 * D], wmod_ref.at[:, 0:2 * D], sems.at[NR])
        cp_mod_b = pltpu.make_async_copy(wmod_hbm.at[:, 2 * D:6 * D], wmod_ref.at[:, 2 * D:6 * D],
                                         sems.at[NR + 1])
        cp_qkv = pltpu.make_async_copy(wqkv_hbm, wqkv_ref, sems.at[NR + 2])
        cp_wo = pltpu.make_async_copy(wo_hbm, wo_ref, sems.at[NR + 3])
        cp_w1 = pltpu.make_async_copy(w1_hbm, w1_ref, sems.at[NR + 4])
        cp_w2 = pltpu.make_async_copy(w2_hbm, w2_ref, sems.at[NR + 5])

        rowh = lax.broadcasted_iota(jnp.int32, (128, TQ), 0) // DH

        def step(qb, ha, hb, s_a, m_a, s_b, m_b):
            if ha is not None:
                g = ha // 8
                j = ha % 8
                if isinstance(g, int):
                    qg = qt_scr[qb, g * 128:(g + 1) * 128, :]
                else:
                    qg = qt_scr[qb, pl.ds(pl.multiple_of(g * 128, 128), 128), :]
                w = jnp.where(rowh == j, qg, jnp.zeros_like(qg))
            if hb is not None:
                mb = m_b[...]
            mx = None
            o = None
            l = None
            for cc in range(NC + abs(SKEW)):
                ca_ = cc - max(SKEW, 0)
                cb_ = cc - max(-SKEW, 0)
                if ha is not None and 0 <= ca_ < NC:
                    c = ca_
                    s = jnp.dot(k_scr[g, c * TK:(c + 1) * TK, :], w,
                                preferred_element_type=jnp.float32)
                    s_a[c * TK:(c + 1) * TK, :] = s
                    mc = jnp.max(s.reshape(TK // 8, 8, TQ), axis=0)
                    mx = mc if mx is None else jnp.maximum(mx, mc)
                if hb is not None and 0 <= cb_ < NC:
                    c = cb_
                    p = jnp.exp2(s_b[c * TK:(c + 1) * TK, :] - mb)
                    lc = jnp.sum(p.reshape(TK // 8, 8, TQ), axis=0)
                    l = lc if l is None else l + lc
                    oc = jnp.dot(vt_scr[hb, :, c * TK:(c + 1) * TK], p.astype(jnp.bfloat16),
                                 preferred_element_type=jnp.float32)
                    o = oc if o is None else o + oc
            if ha is not None:
                m_a[...] = jnp.max(mx, axis=0, keepdims=True)
            if hb is not None:
                on = o / jnp.sum(l, axis=0, keepdims=True)
                if isinstance(hb, int):
                    ot_scr[hb * DH:(hb + 1) * DH, :] = on
                else:
                    ot_scr[pl.ds(pl.multiple_of(hb * DH, DH), DH), :] = on

        @pl.when(i == 0)
        def _prologue():
            cp_mod_a.start()
            x_copy(0).start()
            cp_qkv.start()
            for r in range(1, NR):
                x_copy(r).start()

            c = c_ref[...].astype(jnp.float32)
            sc = c * jax.nn.sigmoid(c)
            sc8 = jnp.broadcast_to(sc, (8, D)).astype(jnp.bfloat16)
            cp_mod_a.wait()
            mod_scr[:, 0:2 * D] = jnp.dot(sc8, wmod_ref[:, 0:2 * D], preferred_element_type=jnp.float32)
            sa = mod_scr[0:1, 0:D]
            ca = mod_scr[0:1, D:2 * D]
            cp_qkv.wait()
            cp_mod_b.start()
            cp_wo.start()
            cp_w1.start()
            cp_w2.start()
            wq_t = wqkv_ref[:, 0:D].astype(jnp.float32).T.astype(jnp.bfloat16)
            wv_t = wqkv_ref[:, 2 * D:3 * D].astype(jnp.float32).T.astype(jnp.bfloat16)
            wk = wqkv_ref[:, D:2 * D]
            for r in range(NR):
                x_copy(r).wait()
                xr = x_ref[r * RC:(r + 1) * RC, :].astype(jnp.float32)
                h = (_ln(xr) * (1.0 + ca) + sa).astype(jnp.bfloat16)
                kk = jnp.dot(h, wk, preferred_element_type=jnp.float32).astype(jnp.bfloat16)
                for g in range(4):
                    k_scr[g, r * RC:(r + 1) * RC, :] = kk[:, g * 128:(g + 1) * 128]
                qt = lax.dot_general(wq_t, h, (((1,), (1,)), ((), ())),
                                     preferred_element_type=jnp.float32)
                qt = (qt * (DH ** -0.5 * LOG2E)).astype(jnp.bfloat16)
                if RC >= TQ:
                    for b in range(RC // TQ):
                        qt_scr[r * (RC // TQ) + b] = qt[:, b * TQ:(b + 1) * TQ]
                else:
                    qt_scr[(r * RC) // TQ, :, (r * RC) % TQ:(r * RC) % TQ + RC] = qt
                vt = lax.dot_general(wv_t, h, (((1,), (1,)), ((), ())),
                                     preferred_element_type=jnp.float32).astype(jnp.bfloat16)
                for hh in range(H):
                    vt_scr[hh, :, r * RC:(r + 1) * RC] = vt[hh * DH:(hh + 1) * DH, :]
            cp_mod_b.wait()
            mod_scr[:, 2 * D:6 * D] = jnp.dot(sc8, wmod_ref[:, 2 * D:6 * D],
                                              preferred_element_type=jnp.float32)
            for v in range(G):
                step(0, v, None, bufs[v][0], bufs[v][1], None, None)

        def body(t, carry):
            for u in range(2):
                @pl.when(t >= -u)
                def _():
                    for v in range(G):
                        hb = (t * 2 + u) * G + v
                        n = hb + G
                        qb = jnp.minimum(i + n // H, NQ - 1)
                        ha = n % H
                        cur = bufs[u * G + v]
                        nxt = bufs[(1 - u) * G + v]
                        step(qb, ha, hb, nxt[0], nxt[1], cur[0], cur[1])
            return carry

        lax.fori_loop(0, NIT, body, 0)

        @pl.when(i == 0)
        def _():
            cp_wo.wait()
            cp_w1.wait()
            cp_w2.wait()

        ga = mod_scr[0:1, 2 * D:3 * D]
        sb = mod_scr[0:1, 3 * D:4 * D]
        cb = mod_scr[0:1, 4 * D:5 * D]
        gb = mod_scr[0:1, 5 * D:6 * D]
        o_att = ot_scr[...].T.astype(jnp.bfloat16)
        a = jnp.dot(o_att, wo_ref[...], preferred_element_type=jnp.float32)
        q0 = pl.multiple_of(i * TQ, TQ)
        x = x_ref[pl.ds(q0, TQ), :].astype(jnp.float32)
        x1 = x + ga * a
        h2 = (_ln(x1) * (1.0 + cb) + sb).astype(jnp.bfloat16)
        b1 = b1_ref[...].astype(jnp.float32).reshape(1, F)
        b2 = b2_ref[...].astype(jnp.float32).reshape(1, D)
        u = jnp.dot(h2, w1_ref[...], preferred_element_type=jnp.float32) + b1
        u = jnp.maximum(u, 0.0)
        u = (u * u).astype(jnp.bfloat16)
        y = jnp.dot(u, w2_ref[...], preferred_element_type=jnp.float32) + b2
        o_ref[0] = (x1 + gb * y).astype(o_ref.dtype)

    def full(shape):
        n = len(shape)
        return pl.BlockSpec(shape, lambda i: (0,) * n)

    hbm = pl.BlockSpec(memory_space=pl.ANY)

    @jax.jit
    def f(A_x, A_wqkv, A_wo, B_x, B_w1, B_b1, B_w2, B_b2, c, w_mod):
        if ONED:
            b1, b2 = B_b1, B_b2
        else:
            b1 = B_b1.reshape(1, F)
            b2 = B_b2.reshape(1, D)
        return pl.pallas_call(
            kernel,
            grid=(NQ,),
            in_specs=[hbm, hbm, hbm, hbm, full(b1.shape), hbm, full(b2.shape), full((1, D)), hbm],
            out_specs=pl.BlockSpec((1, TQ, D), lambda i: (0, i, 0)),
            out_shape=jax.ShapeDtypeStruct((1, S, D), jnp.bfloat16),
            scratch_shapes=[
                pltpu.VMEM((S, D), jnp.bfloat16),
                pltpu.VMEM((D, 3 * D), jnp.bfloat16),
                pltpu.VMEM((D, D), jnp.bfloat16),
                pltpu.VMEM((D, F), jnp.bfloat16),
                pltpu.VMEM((F, D), jnp.bfloat16),
                pltpu.VMEM((D, 6 * D), jnp.bfloat16),
                pltpu.SemaphoreType.DMA((NR + 6,)),
                pltpu.VMEM((4, S, 128), jnp.bfloat16),
                pltpu.VMEM((NQ, D, TQ), jnp.bfloat16),
                pltpu.VMEM((H, DH, S), jnp.bfloat16),
                pltpu.VMEM((8, 6 * D), jnp.float32),
                pltpu.VMEM((D, TQ), jnp.float32),
            ] + [pltpu.VMEM((S, TQ), jnp.float32), pltpu.VMEM((1, TQ), jnp.float32)] * (2 * G),
            compiler_params=pltpu.CompilerParams(
                dimension_semantics=("arbitrary",), vmem_limit_bytes=100 * 1024 * 1024),
        )(A_x, A_wqkv, A_wo, B_w1, b1, B_w2, b2, c, w_mod)

    return f


_impl = make_kernel(G=2)


@jax.jit
def pallas_adaLN_cond__mha_block__dense_activation_squared_relu__prompt_kernel(A_x, A_wqkv, A_wo, B_x, B_w1, B_b1, B_w2, B_b2, c, w_mod):
    return _impl(A_x, A_wqkv, A_wo, B_x, B_w1, B_b1, B_w2, B_b2, c, w_mod)
```

```python
import functools
import jax
import jax.numpy as jnp
from jax import lax
import jax.experimental.pallas as pl
import jax.experimental.pallas.tpu as pltpu

S, D, H, DH, F = 2048, 512, 32, 16, 1792
LOG2E = 1.4426950408889634
EPS = 1e-5


def _ln(x):
    m = jnp.mean(x, axis=-1, keepdims=True)
    xc = x - m
    v = jnp.mean(xc * xc, axis=-1, keepdims=True)
    return xc * lax.rsqrt(v + EPS)


def make_kernel(TQ=512, RC=512, TK=128, NIT=None, ONED=True, U=2, SKEW=0, G=2, CHAIN=2):
    NQ = S // TQ
    NC = S // TK
    NR = S // RC
    if NIT is None:
        NIT = H // (2 * G)

    def kernel(x_hbm, wqkv_hbm, wo_hbm, w1_hbm, b1_ref, w2_hbm, b2_ref, c_ref, wmod_hbm,
               o_ref, x_ref, wqkv_ref, wo_ref, w1_ref, w2_ref, wmod_ref, sems,
               k_scr, qt_scr, vt_scr, mod_scr, ot_scr, *sm_scr):
        bufs = [(sm_scr[2 * b], sm_scr[2 * b + 1]) for b in range(2 * G)]
        i = pl.program_id(0)

        def x_copy(r):
            return pltpu.make_async_copy(x_hbm.at[0, r * RC:(r + 1) * RC, :],
                                         x_ref.at[r * RC:(r + 1) * RC, :], sems.at[r])

        cp_mod_a = pltpu.make_async_copy(wmod_hbm.at[:, 0:2 * D], wmod_ref.at[:, 0:2 * D], sems.at[NR])
        cp_mod_b = pltpu.make_async_copy(wmod_hbm.at[:, 2 * D:6 * D], wmod_ref.at[:, 2 * D:6 * D],
                                         sems.at[NR + 1])
        cp_qkv = [pltpu.make_async_copy(wqkv_hbm.at[:, n * D:(n + 1) * D], wqkv_ref.at[:, n * D:(n + 1) * D],
                                        sems.at[NR + 6 + n]) for n in range(3)]
        cp_wo = pltpu.make_async_copy(wo_hbm, wo_ref, sems.at[NR + 3])
        cp_w1 = pltpu.make_async_copy(w1_hbm, w1_ref, sems.at[NR + 4])
        cp_w2 = pltpu.make_async_copy(w2_hbm, w2_ref, sems.at[NR + 5])

        rowh = lax.shift_right_logical(lax.broadcasted_iota(jnp.int32, (128, TQ), 0), 4)

        def step(qb, ha, hb, s_a, m_a, s_b, m_b):
            if ha is not None:
                if isinstance(ha, int):
                    g = ha // 8
                    j = ha % 8
                else:
                    g = lax.shift_right_logical(ha, 3)
                    j = lax.bitwise_and(ha, 7)
                if isinstance(g, int):
                    qg = qt_scr[qb, g * 128:(g + 1) * 128, :]
                else:
                    qg = qt_scr[qb, pl.ds(pl.multiple_of(g * 128, 128), 128), :]
                w = jnp.where(rowh == j, qg, jnp.zeros_like(qg))
            if hb is not None:
                mb = m_b[...]
            mx = None
            o = None
            l = None
            for cc in range(NC + abs(SKEW)):
                ca_ = cc - max(SKEW, 0)
                cb_ = cc - max(-SKEW, 0)
                if ha is not None and 0 <= ca_ < NC:
                    c = ca_
                    s = jnp.dot(k_scr[g, c * TK:(c + 1) * TK, :], w,
                                preferred_element_type=jnp.float32)
                    s_a[c * TK:(c + 1) * TK, :] = s
                    mc = jnp.max(s.reshape(TK // 8, 8, TQ), axis=0)
                    mx = mc if mx is None else jnp.maximum(mx, mc)
                if hb is not None and 0 <= cb_ < NC:
                    c = cb_
                    p = jnp.exp2(s_b[c * TK:(c + 1) * TK, :] - mb)
                    if CHAIN == 0:
                        lc = jnp.sum(p.reshape(TK // 8, 8, TQ), axis=0)
                        l = lc if l is None else l + lc
                    else:
                        for r in range(0, TK // 8, CHAIN):
                            lc = p[r * 8:(r + 1) * 8, :]
                            for r2 in range(1, CHAIN):
                                lc = lc + p[(r + r2) * 8:(r + r2 + 1) * 8, :]
                            l = lc if l is None else l + lc
                    oc = jnp.dot(vt_scr[hb, :, c * TK:(c + 1) * TK], p.astype(jnp.bfloat16),
                                 preferred_element_type=jnp.float32)
                    o = oc if o is None else o + oc
            if ha is not None:
                m_a[...] = jnp.max(mx, axis=0, keepdims=True)
            if hb is not None:
                on = o / jnp.sum(l, axis=0, keepdims=True)
                if isinstance(hb, int):
                    ot_scr[hb * DH:(hb + 1) * DH, :] = on
                else:
                    ot_scr[pl.ds(pl.multiple_of(hb * DH, DH), DH), :] = on

        @pl.when(i == 0)
        def _prologue():
            cp_mod_a.start()
            x_copy(0).start()
            cp_qkv[1].start()
            cp_qkv[0].start()
            cp_qkv[2].start()
            for r in range(1, NR):
                x_copy(r).start()

            c = c_ref[...].astype(jnp.float32)
            sc = c * jax.nn.sigmoid(c)
            sc8 = jnp.broadcast_to(sc, (8, D)).astype(jnp.bfloat16)
            cp_mod_a.wait()
            mod_scr[:, 0:2 * D] = jnp.dot(sc8, wmod_ref[:, 0:2 * D], preferred_element_type=jnp.float32)
            sa = mod_scr[0:1, 0:D]
            ca = mod_scr[0:1, D:2 * D]
            for r in range(NR):
                x_copy(r).wait()
                xr = x_ref[r * RC:(r + 1) * RC, :].astype(jnp.float32)
                h = (_ln(xr) * (1.0 + ca) + sa).astype(jnp.bfloat16)
                if r == 0:
                    cp_qkv[1].wait()
                kk = jnp.dot(h, wqkv_ref[:, D:2 * D], preferred_element_type=jnp.float32).astype(jnp.bfloat16)
                for g in range(4):
                    k_scr[g, r * RC:(r + 1) * RC, :] = kk[:, g * 128:(g + 1) * 128]
                if r == 0:
                    cp_qkv[0].wait()
                    wq_t = wqkv_ref[:, 0:D].astype(jnp.float32).T.astype(jnp.bfloat16)
                qt = lax.dot_general(wq_t, h, (((1,), (1,)), ((), ())),
                                     preferred_element_type=jnp.float32)
                qt = (qt * (DH ** -0.5 * LOG2E)).astype(jnp.bfloat16)
                if RC >= TQ:
                    for b in range(RC // TQ):
                        qt_scr[r * (RC // TQ) + b] = qt[:, b * TQ:(b + 1) * TQ]
                else:
                    qt_scr[(r * RC) // TQ, :, (r * RC) % TQ:(r * RC) % TQ + RC] = qt
                if r == 0:
                    cp_qkv[2].wait()
                    wv_t = wqkv_ref[:, 2 * D:3 * D].astype(jnp.float32).T.astype(jnp.bfloat16)
                    cp_mod_b.start()
                    cp_wo.start()
                    cp_w1.start()
                    cp_w2.start()
                vt = lax.dot_general(wv_t, h, (((1,), (1,)), ((), ())),
                                     preferred_element_type=jnp.float32).astype(jnp.bfloat16)
                for hh in range(H):
                    vt_scr[hh, :, r * RC:(r + 1) * RC] = vt[hh * DH:(hh + 1) * DH, :]
            cp_mod_b.wait()
            mod_scr[:, 2 * D:6 * D] = jnp.dot(sc8, wmod_ref[:, 2 * D:6 * D],
                                              preferred_element_type=jnp.float32)
            for v in range(G):
                step(0, v, None, bufs[v][0], bufs[v][1], None, None)

        def body(t, carry):
            for u in range(2):
                @pl.when(t >= -u)
                def _():
                    for v in range(G):
                        hb = (t * 2 + u) * G + v
                        n = hb + G
                        qb = jnp.minimum(i + lax.shift_right_logical(n, 5), NQ - 1)
                        ha = lax.bitwise_and(n, H - 1)
                        cur = bufs[u * G + v]
                        nxt = bufs[(1 - u) * G + v]
                        step(qb, ha, hb, nxt[0], nxt[1], cur[0], cur[1])
            return carry

        lax.fori_loop(0, NIT, body, 0)

        @pl.when(i == 0)
        def _():
            cp_wo.wait()
            cp_w1.wait()
            cp_w2.wait()

        ga = mod_scr[0:1, 2 * D:3 * D]
        sb = mod_scr[0:1, 3 * D:4 * D]
        cb = mod_scr[0:1, 4 * D:5 * D]
        gb = mod_scr[0:1, 5 * D:6 * D]
        o_att = ot_scr[...].T.astype(jnp.bfloat16)
        a = jnp.dot(o_att, wo_ref[...], preferred_element_type=jnp.float32)
        q0 = pl.multiple_of(i * TQ, TQ)
        x = x_ref[pl.ds(q0, TQ), :].astype(jnp.float32)
        x1 = x + ga * a
        h2 = (_ln(x1) * (1.0 + cb) + sb).astype(jnp.bfloat16)
        b1 = b1_ref[...].astype(jnp.float32).reshape(1, F)
        b2 = b2_ref[...].astype(jnp.float32).reshape(1, D)
        u = jnp.dot(h2, w1_ref[...], preferred_element_type=jnp.float32) + b1
        u = jnp.maximum(u, 0.0)
        u = (u * u).astype(jnp.bfloat16)
        y = jnp.dot(u, w2_ref[...], preferred_element_type=jnp.float32) + b2
        o_ref[0] = (x1 + gb * y).astype(o_ref.dtype)

    def full(shape):
        n = len(shape)
        return pl.BlockSpec(shape, lambda i: (0,) * n)

    hbm = pl.BlockSpec(memory_space=pl.ANY)

    @jax.jit
    def f(A_x, A_wqkv, A_wo, B_x, B_w1, B_b1, B_w2, B_b2, c, w_mod):
        if ONED:
            b1, b2 = B_b1, B_b2
        else:
            b1 = B_b1.reshape(1, F)
            b2 = B_b2.reshape(1, D)
        return pl.pallas_call(
            kernel,
            grid=(NQ,),
            in_specs=[hbm, hbm, hbm, hbm, full(b1.shape), hbm, full(b2.shape), full((1, D)), hbm],
            out_specs=pl.BlockSpec((1, TQ, D), lambda i: (0, i, 0)),
            out_shape=jax.ShapeDtypeStruct((1, S, D), jnp.bfloat16),
            scratch_shapes=[
                pltpu.VMEM((S, D), jnp.bfloat16),
                pltpu.VMEM((D, 3 * D), jnp.bfloat16),
                pltpu.VMEM((D, D), jnp.bfloat16),
                pltpu.VMEM((D, F), jnp.bfloat16),
                pltpu.VMEM((F, D), jnp.bfloat16),
                pltpu.VMEM((D, 6 * D), jnp.bfloat16),
                pltpu.SemaphoreType.DMA((NR + 9,)),
                pltpu.VMEM((4, S, 128), jnp.bfloat16),
                pltpu.VMEM((NQ, D, TQ), jnp.bfloat16),
                pltpu.VMEM((H, DH, S), jnp.bfloat16),
                pltpu.VMEM((8, 6 * D), jnp.float32),
                pltpu.VMEM((D, TQ), jnp.float32),
            ] + [pltpu.VMEM((S, TQ), jnp.float32), pltpu.VMEM((1, TQ), jnp.float32)] * (2 * G),
            compiler_params=pltpu.CompilerParams(
                dimension_semantics=("arbitrary",), vmem_limit_bytes=100 * 1024 * 1024),
        )(A_x, A_wqkv, A_wo, B_w1, b1, B_w2, b2, c, w_mod)

    return f


_impl = make_kernel()


@jax.jit
def pallas_adaLN_cond__mha_block__dense_activation_squared_relu__prompt_kernel(A_x, A_wqkv, A_wo, B_x, B_w1, B_b1, B_w2, B_b2, c, w_mod):
    return _impl(A_x, A_wqkv, A_wo, B_x, B_w1, B_b1, B_w2, B_b2, c, w_mod)
```

```python
import jax
import jax.numpy as jnp
from jax import lax
import jax.experimental.pallas as pl
import jax.experimental.pallas.tpu as pltpu

S, D, H, DH, F = 2048, 512, 32, 16, 1792
LOG2E = 1.4426950408889634
EPS = 1e-5

TQ = 512
RC = 512
TK = 128
G = 2
NQ = S // TQ
NC = S // TK
NR = S // RC


def _ln(x):
    m = jnp.mean(x, axis=-1, keepdims=True)
    xc = x - m
    v = jnp.mean(xc * xc, axis=-1, keepdims=True)
    return xc * lax.rsqrt(v + EPS)


def _kernel(x_hbm, wqkv_hbm, wo_hbm, w1_hbm, b1_ref, w2_hbm, b2_ref, c_ref, wmod_hbm,
            o_ref, x_ref, wqkv_ref, wo_ref, w1_ref, w2_ref, wmod_ref, sems,
            k_scr, qt_scr, vt_scr, mod_scr, ot_scr, *sm_scr):
    bufs = [(sm_scr[2 * b], sm_scr[2 * b + 1]) for b in range(2 * G)]
    i = pl.program_id(0)

    def x_copy(r):
        return pltpu.make_async_copy(x_hbm.at[0, r * RC:(r + 1) * RC, :],
                                     x_ref.at[r * RC:(r + 1) * RC, :], sems.at[r])

    cp_mod_a = pltpu.make_async_copy(wmod_hbm.at[:, 0:2 * D], wmod_ref.at[:, 0:2 * D],
                                     sems.at[NR])
    cp_mod_b = pltpu.make_async_copy(wmod_hbm.at[:, 2 * D:6 * D], wmod_ref.at[:, 2 * D:6 * D],
                                     sems.at[NR + 1])
    cp_wo = pltpu.make_async_copy(wo_hbm, wo_ref, sems.at[NR + 2])
    cp_w1 = pltpu.make_async_copy(w1_hbm, w1_ref, sems.at[NR + 3])
    cp_w2 = pltpu.make_async_copy(w2_hbm, w2_ref, sems.at[NR + 4])
    cp_qkv = [pltpu.make_async_copy(wqkv_hbm.at[:, n * D:(n + 1) * D],
                                    wqkv_ref.at[:, n * D:(n + 1) * D],
                                    sems.at[NR + 5 + n]) for n in range(3)]

    rowh = lax.shift_right_logical(lax.broadcasted_iota(jnp.int32, (128, TQ), 0), 4)

    def step(qb, ha, hb, s_a, m_a, s_b, m_b):
        if ha is not None:
            if isinstance(ha, int):
                g = ha // 8
                j = ha % 8
                qg = qt_scr[qb, g * 128:(g + 1) * 128, :]
            else:
                g = lax.shift_right_logical(ha, 3)
                j = lax.bitwise_and(ha, 7)
                qg = qt_scr[qb, pl.ds(pl.multiple_of(g * 128, 128), 128), :]
            w = jnp.where(rowh == j, qg, jnp.zeros_like(qg))
        if hb is not None:
            mb = m_b[...]
        mx = None
        o = None
        l = None
        for c in range(NC):
            if ha is not None:
                s = jnp.dot(k_scr[g, c * TK:(c + 1) * TK, :], w,
                            preferred_element_type=jnp.float32)
                s_a[c * TK:(c + 1) * TK, :] = s
                mc = jnp.max(s.reshape(TK // 8, 8, TQ), axis=0)
                mx = mc if mx is None else jnp.maximum(mx, mc)
            if hb is not None:
                p = jnp.exp2(s_b[c * TK:(c + 1) * TK, :] - mb)
                for r in range(0, TK // 8, 2):
                    lc = p[r * 8:(r + 1) * 8, :] + p[(r + 1) * 8:(r + 2) * 8, :]
                    l = lc if l is None else l + lc
                oc = jnp.dot(vt_scr[hb, :, c * TK:(c + 1) * TK], p.astype(jnp.bfloat16),
                             preferred_element_type=jnp.float32)
                o = oc if o is None else o + oc
        if ha is not None:
            m_a[...] = jnp.max(mx, axis=0, keepdims=True)
        if hb is not None:
            on = o / jnp.sum(l, axis=0, keepdims=True)
            if isinstance(hb, int):
                ot_scr[hb * DH:(hb + 1) * DH, :] = on
            else:
                ot_scr[pl.ds(pl.multiple_of(hb * DH, DH), DH), :] = on

    @pl.when(i == 0)
    def _prologue():
        cp_mod_a.start()
        x_copy(0).start()
        cp_qkv[1].start()
        cp_qkv[0].start()
        cp_qkv[2].start()
        for r in range(1, NR):
            x_copy(r).start()

        c = c_ref[...].astype(jnp.float32)
        sc = c * jax.nn.sigmoid(c)
        sc8 = jnp.broadcast_to(sc, (8, D)).astype(jnp.bfloat16)
        cp_mod_a.wait()
        mod_scr[:, 0:2 * D] = jnp.dot(sc8, wmod_ref[:, 0:2 * D],
                                      preferred_element_type=jnp.float32)
        sa = mod_scr[0:1, 0:D]
        ca = mod_scr[0:1, D:2 * D]
        for r in range(NR):
            x_copy(r).wait()
            xr = x_ref[r * RC:(r + 1) * RC, :].astype(jnp.float32)
            h = (_ln(xr) * (1.0 + ca) + sa).astype(jnp.bfloat16)
            if r == 0:
                cp_qkv[1].wait()
            kk = jnp.dot(h, wqkv_ref[:, D:2 * D],
                         preferred_element_type=jnp.float32).astype(jnp.bfloat16)
            for g in range(4):
                k_scr[g, r * RC:(r + 1) * RC, :] = kk[:, g * 128:(g + 1) * 128]
            if r == 0:
                cp_qkv[0].wait()
                wq_t = wqkv_ref[:, 0:D].astype(jnp.float32).T.astype(jnp.bfloat16)
            qt = lax.dot_general(wq_t, h, (((1,), (1,)), ((), ())),
                                 preferred_element_type=jnp.float32)
            qt_scr[r] = (qt * (DH ** -0.5 * LOG2E)).astype(jnp.bfloat16)
            if r == 0:
                cp_qkv[2].wait()
                wv_t = wqkv_ref[:, 2 * D:3 * D].astype(jnp.float32).T.astype(jnp.bfloat16)
                cp_mod_b.start()
                cp_wo.start()
                cp_w1.start()
                cp_w2.start()
            vt = lax.dot_general(wv_t, h, (((1,), (1,)), ((), ())),
                                 preferred_element_type=jnp.float32).astype(jnp.bfloat16)
            for hh in range(H):
                vt_scr[hh, :, r * RC:(r + 1) * RC] = vt[hh * DH:(hh + 1) * DH, :]
        cp_mod_b.wait()
        mod_scr[:, 2 * D:6 * D] = jnp.dot(sc8, wmod_ref[:, 2 * D:6 * D],
                                          preferred_element_type=jnp.float32)
        for v in range(G):
            step(0, v, None, bufs[v][0], bufs[v][1], None, None)

    def body(t, carry):
        for u in range(2):
            nblk = i * (H // G) + t * 2 + u
            last = NQ * (H // G) - 1

            @pl.when(nblk < last)
            def _():
                for v in range(G):
                    hb = (t * 2 + u) * G + v
                    n = hb + G
                    qb = i + lax.shift_right_logical(n, 5)
                    ha = lax.bitwise_and(n, H - 1)
                    cur = bufs[u * G + v]
                    nxt = bufs[(1 - u) * G + v]
                    step(qb, ha, hb, nxt[0], nxt[1], cur[0], cur[1])

            if u == 1:
                @pl.when(nblk == last)
                def _():
                    for v in range(G):
                        cur = bufs[u * G + v]
                        step(None, None, H - G + v, None, None, cur[0], cur[1])
        return carry

    lax.fori_loop(0, H // (2 * G), body, 0)

    @pl.when(i == 0)
    def _():
        cp_wo.wait()
        cp_w1.wait()
        cp_w2.wait()

    ga = mod_scr[0:1, 2 * D:3 * D]
    sb = mod_scr[0:1, 3 * D:4 * D]
    cb = mod_scr[0:1, 4 * D:5 * D]
    gb = mod_scr[0:1, 5 * D:6 * D]
    o_att = ot_scr[...].T.astype(jnp.bfloat16)
    a = jnp.dot(o_att, wo_ref[...], preferred_element_type=jnp.float32)
    q0 = pl.multiple_of(i * TQ, TQ)
    x = x_ref[pl.ds(q0, TQ), :].astype(jnp.float32)
    x1 = x + ga * a
    h2 = (_ln(x1) * (1.0 + cb) + sb).astype(jnp.bfloat16)
    b1 = b1_ref[...].astype(jnp.float32).reshape(1, F)
    b2 = b2_ref[...].astype(jnp.float32).reshape(1, D)
    u = jnp.dot(h2, w1_ref[...], preferred_element_type=jnp.float32) + b1
    u = jnp.maximum(u, 0.0)
    u = (u * u).astype(jnp.bfloat16)
    y = jnp.dot(u, w2_ref[...], preferred_element_type=jnp.float32) + b2
    o_ref[0] = (x1 + gb * y).astype(o_ref.dtype)


def _full(shape):
    n = len(shape)
    return pl.BlockSpec(shape, lambda i: (0,) * n)


@jax.jit
def pallas_adaLN_cond__mha_block__dense_activation_squared_relu__prompt_kernel(
    A_x: jax.Array,
    A_wqkv: jax.Array,
    A_wo: jax.Array,
    B_x: jax.Array,
    B_w1: jax.Array,
    B_b1: jax.Array,
    B_w2: jax.Array,
    B_b2: jax.Array,
    c: jax.Array,
    w_mod: jax.Array,
):
    hbm = pl.BlockSpec(memory_space=pl.ANY)
    return pl.pallas_call(
        _kernel,
        grid=(NQ,),
        in_specs=[hbm, hbm, hbm, hbm, _full((F,)), hbm, _full((D,)), _full((1, D)), hbm],
        out_specs=pl.BlockSpec((1, TQ, D), lambda i: (0, i, 0)),
        out_shape=jax.ShapeDtypeStruct((1, S, D), jnp.bfloat16),
        scratch_shapes=[
            pltpu.VMEM((S, D), jnp.bfloat16),
            pltpu.VMEM((D, 3 * D), jnp.bfloat16),
            pltpu.VMEM((D, D), jnp.bfloat16),
            pltpu.VMEM((D, F), jnp.bfloat16),
            pltpu.VMEM((F, D), jnp.bfloat16),
            pltpu.VMEM((D, 6 * D), jnp.bfloat16),
            pltpu.SemaphoreType.DMA((NR + 8,)),
            pltpu.VMEM((4, S, 128), jnp.bfloat16),
            pltpu.VMEM((NQ, D, TQ), jnp.bfloat16),
            pltpu.VMEM((H, DH, S), jnp.bfloat16),
            pltpu.VMEM((8, 6 * D), jnp.float32),
            pltpu.VMEM((D, TQ), jnp.float32),
        ] + [pltpu.VMEM((S, TQ), jnp.float32), pltpu.VMEM((1, TQ), jnp.float32)] * (2 * G),
        compiler_params=pltpu.CompilerParams(
            dimension_semantics=("arbitrary",), vmem_limit_bytes=100 * 1024 * 1024),
    )(A_x, A_wqkv, A_wo, B_w1, B_b1, B_w2, B_b2, c, w_mod)
```
